```python
import os as _os
_os.environ.setdefault("JAX_PLATFORMS", "cpu")
import jax
import jax.numpy as jnp

def _softmax(x, axis=-1):
    return jax.nn.softmax(x, axis=axis)
def _gelu(x):
    return jax.nn.gelu(x, approximate=True)
def _silu(x):
    return jax.nn.silu(x)
def _sigmoid(x):
    return jax.nn.sigmoid(x)
def _layernorm(x, axis=-1, eps=1e-5):
    m = jnp.mean(x, axis=axis, keepdims=True)
    v = jnp.var(x, axis=axis, keepdims=True)
    return (x - m) / jnp.sqrt(v + eps)
def _scatter_add(tgt, idx, src, axis=0):
    return tgt.at[idx].add(src)
def _segment_sum(src, seg, n):
    return jax.ops.segment_sum(src, seg, n)
class _Rng:
    def __init__(self, key):
        self._k = key
    def _next(self):
        self._k, sub = jax.random.split(self._k)
        return sub
    def normal(self, shape):
        return jax.random.normal(self._next(), shape, dtype=jnp.bfloat16)
    def randint(self, lo, hi, shape):
        return jax.random.randint(self._next(), shape, lo, hi, dtype=jnp.int32)
    def uniform(self, shape, lo=0.0, hi=1.0):
        return jax.random.uniform(self._next(), shape, jnp.bfloat16, lo, hi)
    def permutation(self, n):
        return jax.random.permutation(self._next(), n)


kernel_name = 'parallel_sum__sliding_local_dilated__geglu_ffn__prompt'

def setup_inputs():
    _rng = _Rng(jax.random.key(int.from_bytes(__import__("os").urandom(4), "little")))
    _w = (lambda a: (lambda t: t.astype(jnp.bfloat16) if jnp.issubdtype(t.dtype, jnp.floating) else t)(jnp.asarray(a)))
    def _A_setup():
        B, S, D = 1, 2048, 512
        return {
            "x": _w((lambda *s: _rng.normal(s) * 0.05)(B, S, D)),
            "wqkv": _w((lambda *s: _rng.normal(s) * 0.05)(D, 3 * D)),
            "wo": _w((lambda *s: _rng.normal(s) * 0.05)(D, D)),
        }
    _A_in = _A_setup()

    def _B_setup():
        B, S, D, F = 1, 2048, 512, 1376
        return {
            "x": _w((lambda *s: _rng.normal(s) * 0.05)(B, S, D)),
            "w_gate": _w((lambda *s: _rng.normal(s) * 0.05)(D, F)),
            "w_up": _w((lambda *s: _rng.normal(s) * 0.05)(D, F)),
            "w_down": _w((lambda *s: _rng.normal(s) * 0.05)(F, D)),
        }
    _B_in = _B_setup()

    return {
        "A_x": _A_in["x"],
        "A_wqkv": _A_in["wqkv"],
        "A_wo": _A_in["wo"],
        "B_x": _B_in["x"],
        "B_w_gate": _B_in["w_gate"],
        "B_w_up": _B_in["w_up"],
        "B_w_down": _B_in["w_down"],
    }

def reference(A_x, A_wqkv, A_wo, B_x, B_w_gate, B_w_up, B_w_down):
    def _A_ref(x, wqkv, wo):
        B, S, D = x.shape
        H = 32; Dh = D // H
        W, dil = 8, 2
        qkv = (lambda x, *d: x.transpose(*d))((x @ wqkv).reshape(B, S, 3, H, Dh), 2, 0, 3, 1, 4)
        q, k, v = qkv[0], qkv[1], qkv[2]
        scale = Dh ** -0.5
        pos = jnp.arange(S)
        off = jnp.arange(W) * dil
        idx = pos[:, None] - off[None, :]
        mask = idx >= 0
        idx_c = jnp.where(mask, idx, 0).reshape(-1)
        kg = k[:, :, idx_c, :].reshape(B, H, S, W, Dh)
        vg = v[:, :, idx_c, :].reshape(B, H, S, W, Dh)
        logits = jnp.einsum("bhsd,bhswd->bhsw", q, kg) * scale
        logits = jnp.where(mask[None, None, :, :], logits, -1e9)
        attn = _softmax(logits, axis=-1)
        o = jnp.einsum("bhsw,bhswd->bhsd", attn, vg)
        return (lambda x, *d: x.transpose(*d))(o, 0, 2, 1, 3).reshape(B, S, D) @ wo

    def _B_ref(x, w_gate, w_up, w_down):
        return (_gelu(x @ w_gate) * (x @ w_up)) @ w_down

    x = A_x
    xn = _layernorm(x, axis=-1)
    return x + _A_ref(xn, A_wqkv, A_wo) + _B_ref(xn, B_w_gate, B_w_up, B_w_down)
```

```python
import os
import functools
import jax
import jax.numpy as jnp
from jax import lax
import jax.experimental.pallas as pl
import jax.experimental.pallas.tpu as pltpu

H = 32
DH = 16
W = 8
DIL = 2
HALO = 16
PITCH = 20
TM = int(os.environ.get("TM", 512))
RC = 8
NCHAIN = int(os.environ.get("NCHAIN", 2))
NXQ = int(os.environ.get("NXQ", 4))
NRC = 2
ROT3 = int(os.environ.get("ROT3", 1))
FCH = [int(v) for v in os.environ.get("FCH", "0,128,384,896,1024,1376").split(",")]
LOG2E = 1.4426950408889634
NT_DIMS = (((1,), (1,)), ((), ()))
F32 = jnp.float32
BF16 = jnp.bfloat16
U32 = jnp.uint32
QR = TM // NCHAIN
LNR = 16


def _pk(x, dt=U32):
    return pltpu.bitcast(x, dt)


def _upk(x):
    return pltpu.bitcast(x, BF16)


def _layernorm(x):
    x = x.astype(F32)
    m = jnp.mean(x, axis=-1, keepdims=True)
    xc = x - m
    var = jnp.mean(xc * xc, axis=-1, keepdims=True)
    return (xc * lax.rsqrt(var + 1e-5)).astype(BF16)


def _permute_rows(src, dst_ref, row0, tmp):
    nt = src.shape[1] // 128
    for j in range(nt):
        for h in range(H):
            tmp[j, h * PITCH:h * PITCH + DH, :] = src[h * DH:(h + 1) * DH, j * 128:(j + 1) * 128]
    for d in range(DH):
        for j in range(nt):
            r = (row0 + d * H) // 2
            dst_ref[r:r + H // 2, j * 128:(j + 1) * 128] = _pk(
                tmp[j, pl.ds(d, H, stride=PITCH), :].astype(BF16))


def _q_slot(r):
    return r % NCHAIN, (r // NCHAIN) * RC


def _ln_slot(k):
    return k % NCHAIN, QR + (k // NCHAIN) * (LNR // 2)


def _attn_chunk(qa, k_sc, v_sc, z, r, first):
    nt = k_sc.shape[0]
    c = (DH ** -0.5) * LOG2E
    r0 = r * RC
    b, lr = _q_slot(r)
    buf = qa[b]
    qs = [buf[j, pl.ds(z + lr, RC), :] for j in range(nt)]
    ls = []
    for w in range(W):
        s0 = HALO + r0 - DIL * w
        p = qs[0] * k_sc[0, s0:s0 + RC, :]
        for j in range(1, nt):
            p = p + qs[j] * k_sc[j, s0:s0 + RC, :]
        if ROT3:
            p = (p + pltpu.roll(p, 64, 1)) + (pltpu.roll(p, 32, 1) + pltpu.roll(p, 96, 1))
        else:
            p = p + pltpu.roll(p, 64, 1)
            p = p + pltpu.roll(p, 32, 1)
        if first and r0 < DIL * w:
            pos = r0 + lax.broadcasted_iota(jnp.int32, (RC, 128), 0)
            p = jnp.where(pos >= DIL * w, p, -4e9)
        ls.append(p)
    mx = functools.reduce(jnp.maximum, ls)
    es = [jnp.exp2((l - mx) * c) for l in ls]
    den = functools.reduce(lambda a, b: a + b, es)
    inv = pl.reciprocal(den, approx=True)
    inv = inv * (2.0 - den * inv)
    for j in range(nt):
        acc = None
        for w in range(W):
            s0 = HALO + r0 - DIL * w
            t = es[w] * v_sc[j, s0:s0 + RC, :]
            acc = t if acc is None else acc + t
        buf[j, lr:lr + RC, :] = acc * inv


def _kernel(x_hbm, wqkv_hbm, wo_hbm, wg_hbm, wu_hbm, wd_hbm, o_hbm,
            x_v, o_v, wqkv_v, wo_v, wg_v, wu_v, wd_v, wqkvT_p, wo_p,
            xn_sc, k_sc, v_sc, h_sc, tmp, z_sm, in_sem, out_sem, *qa):
    S, D = x_v.shape
    F = wg_v.shape[0]
    NT = D // 128
    n = S // TM

    copies = {}
    def add(name, src, dst):
        copies[name] = pltpu.make_async_copy(src, dst, in_sem.at[len(copies)])
    def add_gu(c):
        add(f"g{c}", wg_hbm.at[FCH[c]:FCH[c + 1]], wg_v.at[FCH[c]:FCH[c + 1]])
        add(f"u{c}", wu_hbm.at[FCH[c]:FCH[c + 1]], wu_v.at[FCH[c]:FCH[c + 1]])
    XQ = TM // NXQ
    for q in range(NXQ):
        add(f"x0{q}", x_hbm.at[q * XQ:(q + 1) * XQ], x_v.at[q * XQ:(q + 1) * XQ])
    for c in range(4):
        add_gu(c)
    for t in range(3):
        add(f"w{t}", wqkv_hbm.at[:, t * D:(t + 1) * D], wqkv_v.at[t])
    add_gu(4)
    add("x1", x_hbm.at[TM:2 * TM], x_v.at[TM:2 * TM])
    add("wd", wd_hbm, wd_v)
    add("wo", wo_hbm, wo_v)
    add("x2", x_hbm.at[2 * TM:S], x_v.at[2 * TM:S])
    for cp in copies.values():
        cp.start()
    z_sm[0] = 0

    def wait(*names):
        for nm in names:
            copies[nm].wait()

    HD = D // 2
    OR = TM // NRC

    def out_copy(tile, k):
        if k == 0:
            idx = (pl.ds(tile * TM, TM), pl.ds(0, HD))
        else:
            idx = (pl.ds(tile * TM + (k - 1) * OR, OR), pl.ds(HD, HD))
        return pltpu.make_async_copy(o_v.at[idx], o_hbm.at[idx], out_sem.at[tile * (NRC + 1) + k])

    def gate_up(f0, f1):
        xn = _upk(xn_sc[...])
        g = lax.dot_general(xn, wg_v[f0:f1, :], NT_DIMS, preferred_element_type=F32)
        u = lax.dot_general(xn, wu_v[f0:f1, :], NT_DIMS, preferred_element_type=F32)
        h_sc[:, f0:f1] = _pk((jax.nn.gelu(g, approximate=True) * u).astype(BF16))

    def gate(f0, f1):
        return lax.dot_general(_upk(xn_sc[...]), wg_v[f0:f1, :], NT_DIMS, preferred_element_type=F32)

    def up(g, f0, f1):
        u = lax.dot_general(_upk(xn_sc[...]), wu_v[f0:f1, :], NT_DIMS, preferred_element_type=F32)
        h_sc[:, f0:f1] = _pk((jax.nn.gelu(g, approximate=True) * u).astype(BF16))

    def down(f0, f1):
        return jnp.dot(_upk(h_sc[:, f0:f1]), wd_v[f0:f1, :], preferred_element_type=F32)

    def proj(xn, t):
        hd = D // 2
        y = lax.dot_general(xn, _upk(wqkvT_p[t * hd:(t + 1) * hd, :]), NT_DIMS, preferred_element_type=F32)
        for j in range(NT):
            yj = y[:, j * 128:(j + 1) * 128]
            if t == 0:
                for r in range(TM // RC):
                    b, lr = _q_slot(r)
                    qa[b][j, lr:lr + RC, :] = yj[r * RC:(r + 1) * RC]
            else:
                (k_sc if t == 1 else v_sc)[j, HALO:HALO + TM, :] = yj

    def ln_chunk(next_row0, k):
        xn = _pk(_layernorm(x_v[pl.ds(next_row0 + k * LNR, LNR), :]), F32)
        b, lr = _ln_slot(k)
        for j in range(NT):
            qa[b][j, lr:lr + LNR // 2, :] = xn[:, j * 128:(j + 1) * 128]

    def rest(row0, next_row0, first):
        z = z_sm[0]
        for r in range(TM // RC):
            _attn_chunk(qa, k_sc, v_sc, z, r, first)
            if (r + 1) * RC % LNR == 0:
                ln_chunk(next_row0, (r + 1) * RC // LNR - 1)
        k_sc[:, 0:HALO, :] = k_sc[:, TM:TM + HALO, :]
        v_sc[:, 0:HALO, :] = v_sc[:, TM:TM + HALO, :]

    def finish(tile, y):
        row0 = tile * TM if isinstance(tile, int) else pl.multiple_of(tile * TM, TM)
        cols = []
        for j in range(NT):
            rows = []
            for r in range(TM // RC):
                b, lr = _q_slot(r)
                rows.append(qa[b][j, lr:lr + RC, :])
            cols.append(jnp.concatenate(rows, axis=0))
        a = jnp.concatenate(cols, axis=1).astype(BF16)
        y = jnp.dot(a, _upk(wo_p[...]), preferred_element_type=F32) + y
        o = (x_v[pl.ds(row0, TM), :].astype(F32) + y).astype(o_v.dtype)
        o_v[pl.ds(row0, TM), 0:HD] = o[:, 0:HD]
        out_copy(tile, 0).start()
        for k in range(NRC):
            o_v[pl.ds(row0 + k * OR, OR), HD:D] = o[k * OR:(k + 1) * OR, HD:D]
            out_copy(tile, k + 1).start()

    k_sc[:, 0:HALO, :] = jnp.zeros((NT, HALO, 128), F32)
    v_sc[:, 0:HALO, :] = jnp.zeros((NT, HALO, 128), F32)
    for q in range(NXQ):
        if q == NXQ - 1:
            wait(f"x0{q}", "g0", "u0")
        else:
            wait(f"x0{q}")
        xn_sc[q * XQ // 2:(q + 1) * XQ // 2, :] = _pk(_layernorm(x_v[q * XQ:(q + 1) * XQ, :]))
    gate_up(FCH[0], FCH[1])
    wait("g1", "u1")
    gate_up(FCH[1], FCH[2])
    wait("g2", "u2")
    gate_up(FCH[2], FCH[3])
    wait("g3", "u3", "w0", "w1", "w2")
    gate_up(FCH[3], FCH[4])
    for t in range(3):
        _permute_rows(wqkv_v[t].astype(F32).T, wqkvT_p, t * D, tmp.at[t])
        if t < 2:
            proj(_upk(xn_sc[...]), t)
    wait("g4", "u4", "wd", "wo", "x1")
    proj(_upk(xn_sc[...]), 2)
    _permute_rows(wo_v[...].astype(F32), wo_p, 0, tmp.at[3])
    g = gate(FCH[4], F)
    y = down(0, FCH[4])
    up(g, FCH[4], F)
    rest(0, TM, True)
    y = down(FCH[4], F) + y
    finish(0, y)
    wait("x2")

    def body(i, carry):
        row0 = pl.multiple_of(i * TM, TM)
        nxt = pl.multiple_of(jnp.minimum(row0 + TM, S - TM), TM)
        cols = []
        for j in range(NT):
            rows = []
            for k in range(TM // LNR):
                b, lr = _ln_slot(k)
                rows.append(qa[b][j, lr:lr + LNR // 2, :])
            cols.append(jnp.concatenate(rows, axis=0))
        xnp = jnp.concatenate(cols, axis=1)
        for t in range(3):
            proj(_upk(xnp), t)
        xn_sc[...] = pltpu.bitcast(xnp, U32)
        gate_up(0, F)
        rest(row0, nxt, False)
        finish(i, down(0, F))
        return carry
    lax.fori_loop(1, n, body, 0)

    for i in range(n):
        for k in range(NRC + 1):
            out_copy(i, k).wait()


@jax.jit
def pallas_parallel_sum__sliding_local_dilated__geglu_ffn__prompt_kernel(
    A_x, A_wqkv, A_wo, B_x, B_w_gate, B_w_up, B_w_down):
    B, S, D = A_x.shape
    F = B_w_gate.shape[1]
    x = A_x.reshape(S, D)
    NT = D // 128
    out = pl.pallas_call(
        _kernel,
        in_specs=[pl.BlockSpec(memory_space=pl.ANY)] * 6,
        out_specs=pl.BlockSpec(memory_space=pl.ANY),
        out_shape=jax.ShapeDtypeStruct((S, D), A_x.dtype),
        scratch_shapes=[
            pltpu.VMEM((S, D), BF16),
            pltpu.VMEM((S, D), BF16),
            pltpu.VMEM((3, D, D), BF16),
            pltpu.VMEM((D, D), BF16),
            pltpu.VMEM((F, D), BF16),
            pltpu.VMEM((F, D), BF16),
            pltpu.VMEM((F, D), BF16),
            pltpu.VMEM((3 * D // 2, D), U32),
            pltpu.VMEM((D // 2, D), U32),
            pltpu.VMEM((TM // 2, D), U32),
            pltpu.VMEM((NT, TM + HALO, 128), F32),
            pltpu.VMEM((NT, TM + HALO, 128), F32),
            pltpu.VMEM((TM // 2, F), U32),
            pltpu.VMEM((4, NT, H * PITCH, 128), F32),
            pltpu.SMEM((1,), jnp.int32),
            pltpu.SemaphoreType.DMA((32,)),
            pltpu.SemaphoreType.DMA((S // TM * (NRC + 1),)),
        ] + [pltpu.VMEM((NT, QR + QR // 2, 128), F32) for _ in range(NCHAIN)],
        compiler_params=pltpu.CompilerParams(vmem_limit_bytes=100 * 1024 * 1024),
    )(x, A_wqkv, A_wo, B_w_gate.T, B_w_up.T, B_w_down)
    return out.reshape(B, S, D)
```

```python
import functools

import jax
import jax.numpy as jnp
from jax import lax
import jax.experimental.pallas as pl
import jax.experimental.pallas.tpu as pltpu

H = 32
DH = 16
W = 8
DIL = 2
HALO = 16
PITCH = 20
T0 = 768
TM = 640
TX = max(T0, TM)
RC = 8
LNR = 16
NCHAIN = 2
QR = TX // NCHAIN
QPAD = 24
OR = 128
PLAN = [["x0"], ["x1", "x2"], ["g0", "u0"], ["g1", "u1", "x3"],
        ["x4", "x5", "g2", "g3", "u2", "u3"], ["g4", "g5", "u4", "u5", "w0"]]
LOG2E = 1.4426950408889634
QSCALE = (DH ** -0.5) * LOG2E
GC1 = 0.7978845608028654
GC2 = GC1 * 0.044715
NT_DIMS = (((1,), (1,)), ((), ()))
F32 = jnp.float32
BF16 = jnp.bfloat16
U32 = jnp.uint32


def _bits(x):
    return pltpu.bitcast(x, U32)


def _bf16(x):
    return pltpu.bitcast(x, BF16)


def _f32(x):
    return pltpu.bitcast(x, F32)


def _geglu2(g, u):
    t = jnp.tanh(g * (GC1 + GC2 * (g * g)))
    gu = g * u
    return gu + gu * t


def _layernorm(x):
    x = x.astype(F32)
    m = jnp.mean(x, axis=-1, keepdims=True)
    xc = x - m
    var = jnp.mean(xc * xc, axis=-1, keepdims=True)
    return (xc * lax.rsqrt(var + 1e-5)).astype(BF16)


def _scatter_heads(src, tmp):
    for j in range(src.shape[1] // 128):
        for h in range(H):
            tmp[j, h * PITCH:h * PITCH + DH, :] = src[h * DH:(h + 1) * DH, j * 128:(j + 1) * 128]


def _permute_rows(src, dst_ref, tmp):
    _scatter_heads(src, tmp)
    for d in range(DH):
        for j in range(src.shape[1] // 128):
            dst_ref[d * H // 2:(d + 1) * H // 2, j * 128:(j + 1) * 128] = _bits(
                tmp[j, pl.ds(d, H, stride=PITCH), :].astype(BF16))


def _permute_cols(src_t, dst_ref, col0, tmp):
    _scatter_heads(src_t, tmp)
    dpt = 128 // H
    for c in range(DH // dpt):
        for j in range(src_t.shape[1] // 128):
            blk = jnp.concatenate(
                [tmp[j, pl.ds(c * dpt + d, H, stride=PITCH), :] for d in range(dpt)], axis=0)
            dst_ref[j * 64:(j + 1) * 64, col0 + c * 128:col0 + (c + 1) * 128] = _bits(
                blk.T.astype(BF16))


def _q_slot(r):
    return r % NCHAIN, (r // NCHAIN) * RC


def _ln_slot(k):
    return k % NCHAIN, QR + (k // NCHAIN) * (LNR // 2)


def _attn_chunk(qa, k_sc, v_sc, z, r, first):
    nt = k_sc.shape[0]
    r0 = r * RC
    b, lr = _q_slot(r)
    buf = qa[b]
    qs = [_f32(buf[j, pl.ds(z + lr, RC), :]) for j in range(nt)]
    ls = []
    for w in range(W):
        s0 = HALO + r0 - DIL * w
        p = functools.reduce(jnp.add, [qs[j] * k_sc[j, s0:s0 + RC, :] for j in range(nt)])
        p = ((p + pltpu.roll(p, 32, 1)) + pltpu.roll(p, 64, 1)) + pltpu.roll(p, 96, 1)
        if first and r0 < DIL * w:
            pos = r0 + lax.broadcasted_iota(jnp.int32, (RC, 128), 0)
            p = jnp.where(pos >= DIL * w, p, -1e9 * LOG2E)
        ls.append(p)
    mx = functools.reduce(jnp.maximum, ls)
    es = [jnp.exp2(l - mx) for l in ls]
    den = functools.reduce(jnp.add, es)
    inv = pl.reciprocal(den, approx=True)
    inv = inv * (2.0 - den * inv)
    for j in range(nt):
        ts = [es[w] * v_sc[j, HALO + r0 - DIL * w:HALO + r0 - DIL * w + RC, :] for w in range(W)]
        buf[j, lr:lr + RC, :] = _bits(functools.reduce(jnp.add, ts) * inv)


def _kernel(x_hbm, wqkv_hbm, wo_hbm, wg_hbm, wu_hbm, wd_hbm, o_hbm,
            x_v, o_v, wqkv_v, wo_v, wg_v, wu_v, wd_v, wqkv_p, wo_p,
            xn_sc, k_sc, v_sc, h_sc, tmp, z_sm, in_sem, out_sem, *qa):
    S, D = x_v.shape
    F = wg_v.shape[0]
    NT = D // 128
    HD = D // 2
    F0 = F // 128 * 128
    FB = F - F0

    plan = [[(nm[0], int(nm[1:])) for nm in g] for g in PLAN]
    npair = max(k for g in plan for c, k in g if c == "u") + 1
    FC = npair * 128
    arrs = {"x": (x_hbm, x_v), "g": (wg_hbm, wg_v), "u": (wu_hbm, wu_v)}

    def rows(c, a, b):
        return (arrs[c][0].at[a:b], arrs[c][1].at[a:b])

    def merged(grp):
        runs = []
        for c, k in grp:
            if runs and runs[-1][0] == c and runs[-1][2] == k:
                runs[-1][2] = k + 1
            else:
                runs.append([c, k, k + 1])
        return [(wqkv_hbm, wqkv_v) if c == "w" else rows(c, a * 128, b * 128) for c, a, b in runs]

    groups = [merged(g) for g in plan]
    groups += [[rows("g", FC, F), rows("u", FC, F), rows("x", T0, T0 + TM),
                (wd_hbm, wd_v), (wo_hbm, wo_v)],
               [rows("x", T0 + TM, S)]]
    copies = [[pltpu.make_async_copy(src, dst, in_sem.at[gi]) for src, dst in grp]
              for gi, grp in enumerate(groups)]
    for grp in copies:
        for cp in grp:
            cp.start()
    z_sm[0] = 0

    def wait(gi):
        for cp in copies[gi]:
            cp.wait()

    def out_start(r0, nr, c0):
        idx = (pl.ds(r0, nr), pl.ds(c0, HD))
        pltpu.make_async_copy(o_v.at[idx], o_hbm.at[idx], out_sem.at[0]).start()

    def xn_rows(a, b):
        return _bf16(xn_sc[a // 2:b // 2, :])

    def gate(a, b, f0, f1):
        return lax.dot_general(xn_rows(a, b), wg_v[f0:f1, :], NT_DIMS, preferred_element_type=F32)

    def up(g, a, b, f0, f1):
        u = lax.dot_general(xn_rows(a, b), wu_v[f0:f1, :], NT_DIMS, preferred_element_type=F32)
        h_sc[a // 2:b // 2, f0:f1] = _bits(_geglu2(g, u).astype(BF16))

    def ffn_tail(xn):
        tm = xn.shape[0]
        w = jnp.concatenate([wg_v[F0:F, :], wu_v[F0:F, :]], axis=0)
        rt = lax.dot_general(w, xn, NT_DIMS, preferred_element_type=F32)
        ht = _geglu2(rt[0:FB], rt[FB:2 * FB])
        h = jnp.concatenate([ht, jnp.zeros((128 - FB, tm), F32)], axis=0).T
        h_sc[0:tm // 2, F0:F] = _bits(h.astype(BF16))[:, 0:FB]

    def down(tm, f0, f1):
        return jnp.dot(_bf16(h_sc[0:tm // 2, f0:f1]), wd_v[f0:f1, :], preferred_element_type=F32)

    def proj(xn, t, j0=0, j1=NT):
        tm = xn.shape[0]
        y = jnp.dot(xn, _bf16(wqkv_p[:, t * D + j0 * 128:t * D + j1 * 128]),
                    preferred_element_type=F32)
        for j in range(j0, j1):
            yj = y[:, (j - j0) * 128:(j - j0 + 1) * 128]
            if t == 0:
                for r in range(tm // RC):
                    b, lr = _q_slot(r)
                    qa[b][j, lr:lr + RC, :] = _bits(yj[r * RC:(r + 1) * RC] * QSCALE)
            else:
                (k_sc if t == 1 else v_sc)[j, HALO:HALO + tm, :] = yj

    def gather(slot, n, nrows):
        cols = []
        for j in range(NT):
            parts = []
            for r in range(n):
                b, lr = slot(r)
                parts.append(qa[b][j, lr:lr + nrows, :])
            cols.append(jnp.concatenate(parts, axis=0))
        return jnp.concatenate(cols, axis=1)

    def attention(tm, next_row0, first):
        z = z_sm[0]
        na, nl = tm // RC, TM // LNR
        k = 0
        for r in range(na):
            _attn_chunk(qa, k_sc, v_sc, z, r, first)
            while k < nl and (k + 1) * na <= (r + 1) * nl:
                xn = _bits(_layernorm(x_v[pl.ds(next_row0 + k * LNR, LNR), :]))
                b, lr = _ln_slot(k)
                for j in range(NT):
                    qa[b][j, lr:lr + LNR // 2, :] = xn[:, j * 128:(j + 1) * 128]
                k += 1
        k_sc[:, 0:HALO, :] = k_sc[:, tm:tm + HALO, :]
        v_sc[:, 0:HALO, :] = v_sc[:, tm:tm + HALO, :]

    def finish(row0, tm, y):
        a = _f32(gather(_q_slot, tm // RC, RC)).astype(BF16)
        y = jnp.dot(a, _bf16(wo_p[...]), preferred_element_type=F32) + 0.5 * y
        o = (x_v[pl.ds(row0, tm), :].astype(F32) + y).astype(o_v.dtype)
        o_v[pl.ds(row0, tm), 0:HD] = o[:, 0:HD]
        out_start(row0, tm, 0)
        for a0 in range(0, tm, OR):
            o_v[pl.ds(row0 + a0, OR), HD:D] = o[a0:a0 + OR, HD:D]
            out_start(row0 + a0, OR, HD)

    k_sc[:, 0:HALO, :] = jnp.zeros((NT, HALO, 128), F32)
    v_sc[:, 0:HALO, :] = jnp.zeros((NT, HALO, 128), F32)
    nrows = 0
    have = set()
    done = [0] * npair
    for gi, grp in enumerate(plan):
        wait(gi)
        old = nrows
        have |= set(grp)
        nrows = max([nrows] + [(k + 1) * 128 for c, k in grp if c == "x"])
        if nrows > old:
            xn_sc[old // 2:nrows // 2, :] = _bits(_layernorm(x_v[old:nrows, :]))
        for hi in (old, nrows):
            for p in range(npair):
                if ("u", p) in have and done[p] < hi:
                    f0, f1 = p * 128, (p + 1) * 128
                    up(gate(done[p], hi, f0, f1), done[p], hi, f0, f1)
                    done[p] = hi
    assert nrows == T0
    for t in range(3):
        _permute_cols(wqkv_v[:, t * D:(t + 1) * D].astype(F32).T, wqkv_p, t * D, tmp.at[t])
        if t < 2:
            proj(xn_rows(0, T0), t)
    wait(len(plan))
    proj(xn_rows(0, T0), 2, 0, 1)
    ffn_tail(xn_rows(0, T0))
    proj(xn_rows(0, T0), 2, 1, NT)
    _permute_rows(wo_v[...].astype(F32), wo_p, tmp.at[3])
    g = gate(0, T0, FC, F0)
    y = down(T0, 0, FC)
    up(g, 0, T0, FC, F0)
    attention(T0, T0, True)
    y = down(T0, FC, F) + y
    finish(0, T0, y)
    wait(len(plan) + 1)

    def body(i, carry):
        row0 = pl.multiple_of(T0 + i * TM, 128)
        nxt = pl.multiple_of(jnp.minimum(row0 + TM, S - TM), 128)
        xnp = gather(_ln_slot, TM // LNR, LNR // 2)
        proj(_bf16(xnp), 0)
        ffn_tail(_bf16(xnp))
        proj(_bf16(xnp), 1)
        proj(_bf16(xnp), 2)
        xn_sc[0:TM // 2, :] = xnp
        up(gate(0, TM, 0, F0), 0, TM, 0, F0)
        attention(TM, nxt, False)
        finish(row0, TM, down(TM, 0, F))
        return carry

    lax.fori_loop(0, (S - T0) // TM, body, 0)

    pltpu.make_async_copy(o_v, o_hbm, out_sem.at[0]).wait()


@jax.jit
def pallas_parallel_sum__sliding_local_dilated__geglu_ffn__prompt_kernel(
    A_x: jax.Array,
    A_wqkv: jax.Array,
    A_wo: jax.Array,
    B_x: jax.Array,
    B_w_gate: jax.Array,
    B_w_up: jax.Array,
    B_w_down: jax.Array,
):
    B, S, D = A_x.shape
    F = B_w_gate.shape[1]
    assert B == 1 and D == H * DH and (S - T0) % TM == 0 and S > T0 + TM
    NT = D // 128
    out = pl.pallas_call(
        _kernel,
        in_specs=[pl.BlockSpec(memory_space=pl.ANY)] * 6,
        out_specs=pl.BlockSpec(memory_space=pl.ANY),
        out_shape=jax.ShapeDtypeStruct((S, D), A_x.dtype),
        scratch_shapes=[
            pltpu.VMEM((S, D), BF16),
            pltpu.VMEM((S, D), BF16),
            pltpu.VMEM((D, 3 * D), BF16),
            pltpu.VMEM((D, D), BF16),
            pltpu.VMEM((F, D), BF16),
            pltpu.VMEM((F, D), BF16),
            pltpu.VMEM((F, D), BF16),
            pltpu.VMEM((D // 2, 3 * D), U32),
            pltpu.VMEM((D // 2, D), U32),
            pltpu.VMEM((TX // 2, D), U32),
            pltpu.VMEM((NT, TX + HALO, 128), F32),
            pltpu.VMEM((NT, TX + HALO, 128), F32),
            pltpu.VMEM((TX // 2, F), U32),
            pltpu.VMEM((4, NT, H * PITCH, 128), F32),
            pltpu.SMEM((1,), jnp.int32),
            pltpu.SemaphoreType.DMA((len(PLAN) + 2,)),
            pltpu.SemaphoreType.DMA((1,)),
        ] + [pltpu.VMEM((NT, QR + TM // (2 * NCHAIN) + QPAD, 128), U32)
             for _ in range(NCHAIN)],
        compiler_params=pltpu.CompilerParams(
            vmem_limit_bytes=100 * 1024 * 1024,
            disable_bounds_checks=True,
            disable_semaphore_checks=True),
    )(A_x.reshape(S, D), A_wqkv, A_wo, B_w_gate.T, B_w_up.T, B_w_down)
    return out.reshape(B, S, D)
```

```python
import functools

import jax
import jax.numpy as jnp
from jax import lax
import jax.experimental.pallas as pl
import jax.experimental.pallas.tpu as pltpu

H = 32
DH = 16
W = 8
DIL = 2
HALO = 16
PITCH = 20
T0 = 768
TM = 640
TX = max(T0, TM)
RC = 8
LNR = 16
NCHAIN = 2
QR = TX // NCHAIN
SPARE = QR + TM // (2 * NCHAIN)
QPAD = 24
TRIG = 4
OR = 64
PLAN = [["x0"], ["x1", "x2"], ["g0", "u0"], ["g1", "u1", "x3"],
        ["x4", "x5", "g2", "g3", "u2", "u3"], ["g4", "g5", "u4", "u5", "w0"]]
LOG2E = 1.4426950408889634
QSCALE = (DH ** -0.5) * LOG2E
GC1 = 0.7978845608028654
GC2 = GC1 * 0.044715
NT_DIMS = (((1,), (1,)), ((), ()))
F32 = jnp.float32
BF16 = jnp.bfloat16
U32 = jnp.uint32


def _bits(x):
    return pltpu.bitcast(x, U32)


def _bf16(x):
    return pltpu.bitcast(x, BF16)


def _f32(x):
    return pltpu.bitcast(x, F32)


def _geglu2(g, u):
    t = jnp.tanh(g * (GC1 + GC2 * (g * g)))
    gu = g * u
    return gu + gu * t


def _layernorm(x):
    x = x.astype(F32)
    m = jnp.mean(x, axis=-1, keepdims=True)
    xc = x - m
    var = jnp.mean(xc * xc, axis=-1, keepdims=True)
    return (xc * lax.rsqrt(var + 1e-5)).astype(BF16)


def _scatter_heads(src, tmp):
    for j in range(src.shape[1] // 128):
        for h in range(H):
            tmp[j, h * PITCH:h * PITCH + DH, :] = src[h * DH:(h + 1) * DH, j * 128:(j + 1) * 128]


def _permute_rows(src, dst_ref, tmp):
    _scatter_heads(src, tmp)
    for d in range(DH):
        for j in range(src.shape[1] // 128):
            dst_ref[d * H // 2:(d + 1) * H // 2, j * 128:(j + 1) * 128] = _bits(
                tmp[j, pl.ds(d, H, stride=PITCH), :].astype(BF16))


def _permute_cols(src_t, dst_ref, col0, tmp):
    _scatter_heads(src_t, tmp)
    dpt = 128 // H
    for c in range(DH // dpt):
        for j in range(src_t.shape[1] // 128):
            blk = jnp.concatenate(
                [tmp[j, pl.ds(c * dpt + d, H, stride=PITCH), :] for d in range(dpt)], axis=0)
            dst_ref[j * 64:(j + 1) * 64, col0 + c * 128:col0 + (c + 1) * 128] = _bits(
                blk.T.astype(BF16))


def _q_slot(r):
    return r % NCHAIN, (r // NCHAIN) * RC


def _ln_slot(k):
    return k % NCHAIN, QR + (k // NCHAIN) * (LNR // 2)


def _attn_chunk(qa, k_sc, v_sc, z, r, first):
    nt = k_sc.shape[0]
    r0 = r * RC
    b, lr = _q_slot(r)
    buf = qa[b]
    qs = [_f32(buf[j, pl.ds(z + lr, RC), :]) for j in range(nt)]
    ls = []
    for w in range(W):
        s0 = HALO + r0 - DIL * w
        p = functools.reduce(jnp.add, [qs[j] * k_sc[j, s0:s0 + RC, :] for j in range(nt)])
        p = ((p + pltpu.roll(p, 32, 1)) + pltpu.roll(p, 64, 1)) + pltpu.roll(p, 96, 1)
        if first and r0 < DIL * w:
            pos = r0 + lax.broadcasted_iota(jnp.int32, (RC, 128), 0)
            p = jnp.where(pos >= DIL * w, p, -1e9 * LOG2E)
        ls.append(p)
        if w == TRIG:
            qa[(b + 1) % NCHAIN][0, SPARE:SPARE + RC, :] = _bits(p)
    mx = functools.reduce(jnp.maximum, ls)
    es = [jnp.exp2(l - mx) for l in ls]
    den = functools.reduce(jnp.add, es)
    inv = pl.reciprocal(den, approx=True)
    inv = inv * (2.0 - den * inv)
    for j in range(nt):
        ts = [es[w] * v_sc[j, HALO + r0 - DIL * w:HALO + r0 - DIL * w + RC, :] for w in range(W)]
        buf[j, lr:lr + RC, :] = _bits(functools.reduce(jnp.add, ts) * inv)


def _kernel(x_hbm, wqkv_hbm, wo_hbm, wg_hbm, wu_hbm, wd_hbm, o_hbm,
            x_v, o_v, wqkv_v, wo_v, wg_v, wu_v, wd_v, wqkv_p, wo_p,
            xn_sc, k_sc, v_sc, h_sc, tmp, z_sm, in_sem, out_sem, *qa):
    S, D = x_v.shape
    F = wg_v.shape[0]
    NT = D // 128
    F0 = F // 128 * 128
    FB = F - F0

    plan = [[(nm[0], int(nm[1:])) for nm in g] for g in PLAN]
    npair = max(k for g in plan for c, k in g if c == "u") + 1
    FC = npair * 128
    arrs = {"x": (x_hbm, x_v), "g": (wg_hbm, wg_v), "u": (wu_hbm, wu_v)}

    def rows(c, a, b):
        return (arrs[c][0].at[a:b], arrs[c][1].at[a:b])

    def merged(grp):
        runs = []
        for c, k in grp:
            if runs and runs[-1][0] == c and runs[-1][2] == k:
                runs[-1][2] = k + 1
            else:
                runs.append([c, k, k + 1])
        return [(wqkv_hbm, wqkv_v) if c == "w" else rows(c, a * 128, b * 128) for c, a, b in runs]

    groups = [merged(g) for g in plan]
    groups += [[rows("g", FC, F), rows("u", FC, F), rows("x", T0, T0 + TM),
                (wd_hbm, wd_v), (wo_hbm, wo_v)],
               [rows("x", T0 + TM, S)]]
    copies = [[pltpu.make_async_copy(src, dst, in_sem.at[gi]) for src, dst in grp]
              for gi, grp in enumerate(groups)]
    for grp in copies:
        for cp in grp:
            cp.start()
    z_sm[0] = 0

    def wait(gi):
        for cp in copies[gi]:
            cp.wait()

    def xn_rows(a, b):
        return _bf16(xn_sc[a // 2:b // 2, :])

    def gate(a, b, f0, f1):
        return lax.dot_general(xn_rows(a, b), wg_v[f0:f1, :], NT_DIMS, preferred_element_type=F32)

    def up(g, a, b, f0, f1):
        u = lax.dot_general(xn_rows(a, b), wu_v[f0:f1, :], NT_DIMS, preferred_element_type=F32)
        h_sc[a // 2:b // 2, f0:f1] = _bits(_geglu2(g, u).astype(BF16))

    def ffn_tail(xn):
        tm = xn.shape[0]
        w = jnp.concatenate([wg_v[F0:F, :], wu_v[F0:F, :]], axis=0)
        rt = lax.dot_general(w, xn, NT_DIMS, preferred_element_type=F32)
        ht = _geglu2(rt[0:FB], rt[FB:2 * FB])
        h = jnp.concatenate([ht, jnp.zeros((128 - FB, tm), F32)], axis=0).T
        h_sc[0:tm // 2, F0:F] = _bits(h.astype(BF16))[:, 0:FB]

    def down(tm, f0, f1):
        return jnp.dot(_bf16(h_sc[0:tm // 2, f0:f1]), wd_v[f0:f1, :], preferred_element_type=F32)

    def proj(xn, t, j0=0, j1=NT):
        tm = xn.shape[0]
        y = jnp.dot(xn, _bf16(wqkv_p[:, t * D + j0 * 128:t * D + j1 * 128]),
                    preferred_element_type=F32)
        for j in range(j0, j1):
            yj = y[:, (j - j0) * 128:(j - j0 + 1) * 128]
            if t == 0:
                for r in range(tm // RC):
                    b, lr = _q_slot(r)
                    qa[b][j, lr:lr + RC, :] = _bits(yj[r * RC:(r + 1) * RC] * QSCALE)
            else:
                (k_sc if t == 1 else v_sc)[j, HALO:HALO + tm, :] = yj

    def gather(slot, n, nrows):
        cols = []
        for j in range(NT):
            parts = []
            for r in range(n):
                b, lr = slot(r)
                parts.append(qa[b][j, lr:lr + nrows, :])
            cols.append(jnp.concatenate(parts, axis=0))
        return jnp.concatenate(cols, axis=1)

    def attention(tm, next_row0, first):
        z = z_sm[0]
        na, nl = tm // RC, TM // LNR
        k = 0
        for r in range(na):
            _attn_chunk(qa, k_sc, v_sc, z, r, first)
            while k < nl and (k + 1) * na <= (r + 1) * nl:
                xn = _bits(_layernorm(x_v[pl.ds(next_row0 + k * LNR, LNR), :]))
                b, lr = _ln_slot(k)
                for j in range(NT):
                    qa[b][j, lr:lr + LNR // 2, :] = xn[:, j * 128:(j + 1) * 128]
                k += 1
        k_sc[:, 0:HALO, :] = k_sc[:, tm:tm + HALO, :]
        v_sc[:, 0:HALO, :] = v_sc[:, tm:tm + HALO, :]

    def finish(row0, tm, y):
        a = _f32(gather(_q_slot, tm // RC, RC)).astype(BF16)
        y = jnp.dot(a, _bf16(wo_p[...]), preferred_element_type=F32) + 0.5 * y

        def emit(a0, a1, c0, c1):
            idx = (pl.ds(row0 + a0, a1 - a0), pl.ds(c0, c1 - c0))
            o_v[idx] = (x_v[idx].astype(F32) + y[a0:a1, c0:c1]).astype(o_v.dtype)
            pltpu.make_async_copy(o_v.at[idx], o_hbm.at[idx], out_sem.at[0]).start()

        emit(0, tm, 0, D // 2)
        emit(0, tm, D // 2, D - 128)
        for a0 in range(0, tm, OR):
            emit(a0, a0 + OR, D - 128, D)

    def whole(i_, carry_):
        k_sc[:, 0:HALO, :] = jnp.zeros((NT, HALO, 128), F32)
        v_sc[:, 0:HALO, :] = jnp.zeros((NT, HALO, 128), F32)
        nrows = 0
        have = set()
        done = [0] * npair
        for gi, grp in enumerate(plan):
            wait(gi)
            old = nrows
            have |= set(grp)
            nrows = max([nrows] + [(k + 1) * 128 for c, k in grp if c == "x"])
            if nrows > old:
                xn_sc[old // 2:nrows // 2, :] = _bits(_layernorm(x_v[old:nrows, :]))
            for hi in (old, nrows):
                for p in range(npair):
                    if ("u", p) in have and done[p] < hi:
                        f0, f1 = p * 128, (p + 1) * 128
                        up(gate(done[p], hi, f0, f1), done[p], hi, f0, f1)
                        done[p] = hi
        assert nrows == T0
        for t in (1, 2, 0):
            _permute_cols(wqkv_v[:, t * D:(t + 1) * D].astype(F32).T, wqkv_p, t * D, tmp.at[t])
            if t > 0:
                proj(xn_rows(0, T0), t)
        wait(len(plan))
        proj(xn_rows(0, T0), 0, 0, 1)
        ffn_tail(xn_rows(0, T0))
        proj(xn_rows(0, T0), 0, 1, NT)
        _permute_rows(wo_v[...].astype(F32), wo_p, tmp.at[3])
        g = gate(0, T0, FC, F0)
        y = down(T0, 0, FC)
        up(g, 0, T0, FC, F0)
        attention(T0, T0, True)
        y = down(T0, FC, F) + y
        finish(0, T0, y)
        wait(len(plan) + 1)

        def body(i, carry):
            row0 = pl.multiple_of(T0 + i * TM, 128)
            nxt = pl.multiple_of(jnp.minimum(row0 + TM, S - TM), 128)
            xnp = gather(_ln_slot, TM // LNR, LNR // 2)
            proj(_bf16(xnp), 0)
            ffn_tail(_bf16(xnp))
            proj(_bf16(xnp), 1)
            proj(_bf16(xnp), 2)
            xn_sc[0:TM // 2, :] = xnp
            up(gate(0, TM, 0, F0), 0, TM, 0, F0)
            attention(TM, nxt, False)
            finish(row0, TM, down(TM, 0, F))
            return carry

        lax.fori_loop(0, (S - T0) // TM, body, 0)
        return carry_

    lax.fori_loop(0, z_sm[0] + 1, whole, 0)

    pltpu.make_async_copy(o_v, o_hbm, out_sem.at[0]).wait()


@jax.jit
def pallas_parallel_sum__sliding_local_dilated__geglu_ffn__prompt_kernel(
    A_x: jax.Array,
    A_wqkv: jax.Array,
    A_wo: jax.Array,
    B_x: jax.Array,
    B_w_gate: jax.Array,
    B_w_up: jax.Array,
    B_w_down: jax.Array,
):
    B, S, D = A_x.shape
    F = B_w_gate.shape[1]
    assert B == 1 and D == H * DH and (S - T0) % TM == 0 and S > T0 + TM
    NT = D // 128
    out = pl.pallas_call(
        _kernel,
        in_specs=[pl.BlockSpec(memory_space=pl.ANY)] * 6,
        out_specs=pl.BlockSpec(memory_space=pl.ANY),
        out_shape=jax.ShapeDtypeStruct((S, D), A_x.dtype),
        scratch_shapes=[
            pltpu.VMEM((S, D), BF16),
            pltpu.VMEM((S, D), BF16),
            pltpu.VMEM((D, 3 * D), BF16),
            pltpu.VMEM((D, D), BF16),
            pltpu.VMEM((F, D), BF16),
            pltpu.VMEM((F, D), BF16),
            pltpu.VMEM((F, D), BF16),
            pltpu.VMEM((D // 2, 3 * D), U32),
            pltpu.VMEM((D // 2, D), U32),
            pltpu.VMEM((TX // 2, D), U32),
            pltpu.VMEM((NT, TX + HALO, 128), F32),
            pltpu.VMEM((NT, TX + HALO, 128), F32),
            pltpu.VMEM((TX // 2, F), U32),
            pltpu.VMEM((4, NT, H * PITCH, 128), F32),
            pltpu.SMEM((1,), jnp.int32),
            pltpu.SemaphoreType.DMA((len(PLAN) + 2,)),
            pltpu.SemaphoreType.DMA((1,)),
        ] + [pltpu.VMEM((NT, SPARE + QPAD, 128), U32)
             for _ in range(NCHAIN)],
        compiler_params=pltpu.CompilerParams(
            vmem_limit_bytes=100 * 1024 * 1024,
            disable_bounds_checks=True,
            disable_semaphore_checks=True),
    )(A_x.reshape(S, D), A_wqkv, A_wo, B_w_gate.T, B_w_up.T, B_w_down)
    return out.reshape(B, S, D)
```

```python
import functools

import jax
import jax.numpy as jnp
from jax import lax
import jax.experimental.pallas as pl
import jax.experimental.pallas.tpu as pltpu

H = 32
DH = 16
W = 8
DIL = 2
HALO = 16
PITCH = 20
T0 = 768
TM = 640
TX = max(T0, TM)
RC = 8
LNR = 16
NCHAIN = 2
QR = TX // NCHAIN
SPARE = QR + TM // (2 * NCHAIN)
QPAD = 8
TRIG = 3
OR = 64
PLAN = [["x0"], ["x1", "x2"], ["g0", "u0"], ["g1", "u1", "x3"],
        ["x4", "x5", "g2", "g3", "u2", "u3"], ["g4", "g5", "u4", "u5", "w0"]]
LOG2E = 1.4426950408889634
QSCALE = (DH ** -0.5) * LOG2E
GC1 = 0.7978845608028654
GC2 = GC1 * 0.044715
NT_DIMS = (((1,), (1,)), ((), ()))
F32 = jnp.float32
BF16 = jnp.bfloat16
U32 = jnp.uint32


def _bits(x):
    return pltpu.bitcast(x, U32)


def _bf16(x):
    return pltpu.bitcast(x, BF16)


def _f32(x):
    return pltpu.bitcast(x, F32)


def _geglu2(g, u):
    t = jnp.tanh(g * (GC1 + GC2 * (g * g)))
    gu = g * u
    return gu + gu * t


def _layernorm(x):
    x = x.astype(F32)
    m = jnp.mean(x, axis=-1, keepdims=True)
    xc = x - m
    var = jnp.mean(xc * xc, axis=-1, keepdims=True)
    return (xc * lax.rsqrt(var + 1e-5)).astype(BF16)


def _scatter_heads(src, tmp):
    for j in range(src.shape[1] // 128):
        for h in range(H):
            tmp[j, h * PITCH:h * PITCH + DH, :] = src[h * DH:(h + 1) * DH, j * 128:(j + 1) * 128]


def _permute_rows(src, dst_ref, tmp):
    _scatter_heads(src, tmp)
    for d in range(DH):
        for j in range(src.shape[1] // 128):
            dst_ref[d * H // 2:(d + 1) * H // 2, j * 128:(j + 1) * 128] = _bits(
                tmp[j, pl.ds(d, H, stride=PITCH), :].astype(BF16))


def _permute_cols(src_t, dst_ref, col0, tmp):
    _scatter_heads(src_t, tmp)
    dpt = 128 // H
    for c in range(DH // dpt):
        for j in range(src_t.shape[1] // 128):
            blk = jnp.concatenate(
                [tmp[j, pl.ds(c * dpt + d, H, stride=PITCH), :] for d in range(dpt)], axis=0)
            dst_ref[j * 64:(j + 1) * 64, col0 + c * 128:col0 + (c + 1) * 128] = _bits(
                blk.T.astype(BF16))


def _split(x, nrows):
    n = x.shape[0] // (NCHAIN * nrows)
    x = x.reshape(n, NCHAIN, nrows, 128)
    return [x[:, b].reshape(n * nrows, 128) for b in range(NCHAIN)]


def _merge(xs, nrows):
    n = xs[0].shape[0] // nrows
    x = jnp.concatenate([x.reshape(n, 1, nrows, 128) for x in xs], axis=1)
    return x.reshape(n * NCHAIN * nrows, 128)


def _attn_chunk(qa, k_sc, v_sc, z, g, b, masked):
    nt = k_sc.shape[0]
    r0 = (g * NCHAIN + b) * RC
    lr = g * RC
    buf = qa[b]
    qs = [_f32(buf[j, pl.ds(z + lr, RC), :]) for j in range(nt)]
    win = [pl.ds(r0 + (HALO - DIL * w), RC) for w in range(W)]
    ls = []
    for w in range(W):
        p = functools.reduce(jnp.add, [qs[j] * k_sc[j, win[w], :] for j in range(nt)])
        p = ((p + pltpu.roll(p, 32, 1)) + pltpu.roll(p, 64, 1)) + pltpu.roll(p, 96, 1)
        if masked and r0 < DIL * w:
            pos = r0 + lax.broadcasted_iota(jnp.int32, (RC, 128), 0)
            p = jnp.where(pos >= DIL * w, p, -1e9 * LOG2E)
        ls.append(p)
        if w == TRIG:
            qa[(b + 1) % NCHAIN][0, SPARE:SPARE + RC, :] = _bits(p)
    mx = functools.reduce(jnp.maximum, ls)
    es = [jnp.exp2(l - mx) for l in ls]
    den = functools.reduce(jnp.add, es)
    inv = pl.reciprocal(den, approx=True)
    inv = inv * (2.0 - den * inv)
    for j in range(nt):
        acc = functools.reduce(jnp.add, [es[w] * v_sc[j, win[w], :] for w in range(W)])
        buf[j, pl.ds(lr, RC), :] = _bits(acc * inv)


def _kernel(x_hbm, wqkv_hbm, wo_hbm, wg_hbm, wu_hbm, wd_hbm, o_hbm,
            x_v, o_v, wqkv_v, wo_v, wg_v, wu_v, wd_v, wqkv_p, wo_p,
            xn_sc, k_sc, v_sc, h_sc, tmp, z_sm, in_sem, out_sem, *qa):
    S, D = x_v.shape
    F = wg_v.shape[0]
    NT = D // 128
    F0 = F // 128 * 128
    FB = F - F0

    plan = [[(nm[0], int(nm[1:])) for nm in g] for g in PLAN]
    npair = max(k for g in plan for c, k in g if c == "u") + 1
    FC = npair * 128
    arrs = {"x": (x_hbm, x_v), "g": (wg_hbm, wg_v), "u": (wu_hbm, wu_v)}

    def rows(c, a, b):
        return (arrs[c][0].at[a:b], arrs[c][1].at[a:b])

    def merged(grp):
        runs = []
        for c, k in grp:
            if runs and runs[-1][0] == c and runs[-1][2] == k:
                runs[-1][2] = k + 1
            else:
                runs.append([c, k, k + 1])
        return [(wqkv_hbm, wqkv_v) if c == "w" else rows(c, a * 128, b * 128) for c, a, b in runs]

    groups = [merged(g) for g in plan]
    groups += [[rows("g", FC, F), rows("u", FC, F), rows("x", T0, T0 + TM),
                (wd_hbm, wd_v), (wo_hbm, wo_v)],
               [rows("x", T0 + TM, S)]]
    copies = [[pltpu.make_async_copy(src, dst, in_sem.at[gi]) for src, dst in grp]
              for gi, grp in enumerate(groups)]
    for grp in copies:
        for cp in grp:
            cp.start()
    z_sm[0] = 0

    def wait(gi):
        for cp in copies[gi]:
            cp.wait()

    def xn_rows(a, b):
        return _bf16(xn_sc[a // 2:b // 2, :])

    def gate(a, b, f0, f1):
        return lax.dot_general(xn_rows(a, b), wg_v[f0:f1, :], NT_DIMS, preferred_element_type=F32)

    def up(g, a, b, f0, f1):
        u = lax.dot_general(xn_rows(a, b), wu_v[f0:f1, :], NT_DIMS, preferred_element_type=F32)
        h_sc[a // 2:b // 2, f0:f1] = _bits(_geglu2(g, u).astype(BF16))

    def ffn_tail(xn):
        tm = xn.shape[0]
        w = jnp.concatenate([wg_v[F0:F, :], wu_v[F0:F, :]], axis=0)
        rt = lax.dot_general(w, xn, NT_DIMS, preferred_element_type=F32)
        ht = _geglu2(rt[0:FB], rt[FB:2 * FB])
        h = jnp.concatenate([ht, jnp.zeros((128 - FB, tm), F32)], axis=0).T
        h_sc[0:tm // 2, F0:F] = _bits(h.astype(BF16))[:, 0:FB]

    def down(tm, f0, f1):
        return jnp.dot(_bf16(h_sc[0:tm // 2, f0:f1]), wd_v[f0:f1, :], preferred_element_type=F32)

    def proj(xn, t, j0=0, j1=NT):
        tm = xn.shape[0]
        y = jnp.dot(xn, _bf16(wqkv_p[:, t * D + j0 * 128:t * D + j1 * 128]),
                    preferred_element_type=F32)
        for j in range(j0, j1):
            yj = y[:, (j - j0) * 128:(j - j0 + 1) * 128]
            if t == 0:
                for b, part in enumerate(_split(_bits(yj * QSCALE), RC)):
                    qa[b][j, 0:tm // NCHAIN, :] = part
            else:
                (k_sc if t == 1 else v_sc)[j, HALO:HALO + tm, :] = yj

    def gather(row0, n):
        return jnp.concatenate(
            [_merge([qa[b][j, row0:row0 + n, :] for b in range(NCHAIN)], RC) for j in range(NT)],
            axis=1)

    def attention(tm, next_row0, first):
        z = z_sm[0]

        def step(i, with_ln, masked=False):
            for lb in range(NCHAIN):
                g = i * NCHAIN + lb
                for b in range(NCHAIN):
                    _attn_chunk(qa, k_sc, v_sc, z, g, b, masked)
                if with_ln:
                    r = pl.multiple_of(next_row0 + g * LNR, LNR)
                    xn = _bits(_layernorm(x_v[pl.ds(r, LNR), :]))
                    for j in range(NT):
                        qa[lb][j, pl.ds(QR + i * (LNR // 2), LNR // 2), :] = (
                            xn[:, j * 128:(j + 1) * 128])

        def run(lo, hi, with_ln):
            def body(i, carry):
                step(i, with_ln)
                return carry
            if lo < hi:
                lax.fori_loop(lo, hi, body, 0, unroll=True)

        n_ln, n_all = TM // (LNR * NCHAIN), tm // (RC * NCHAIN * NCHAIN)
        if first:
            step(0, True, masked=True)
        run(1 if first else 0, n_ln, True)
        run(n_ln, n_all, False)
        k_sc[:, 0:HALO, :] = k_sc[:, tm:tm + HALO, :]
        v_sc[:, 0:HALO, :] = v_sc[:, tm:tm + HALO, :]

    def finish(row0, tm, y):
        a = _f32(gather(0, tm // NCHAIN)).astype(BF16)
        y = jnp.dot(a, _bf16(wo_p[...]), preferred_element_type=F32) + 0.5 * y

        def emit(a0, a1, c0, c1):
            idx = (pl.ds(row0 + a0, a1 - a0), pl.ds(c0, c1 - c0))
            o_v[idx] = (x_v[idx].astype(F32) + y[a0:a1, c0:c1]).astype(o_v.dtype)
            pltpu.make_async_copy(o_v.at[idx], o_hbm.at[idx], out_sem.at[0]).start()

        emit(0, tm, 0, D // 2)
        emit(0, tm, D // 2, D - 128)
        for a0 in range(0, tm, OR):
            emit(a0, a0 + OR, D - 128, D)

    def whole(i_, carry_):
        k_sc[:, 0:HALO, :] = jnp.zeros((NT, HALO, 128), F32)
        v_sc[:, 0:HALO, :] = jnp.zeros((NT, HALO, 128), F32)
        nrows = 0
        have = set()
        done = [0] * npair
        for gi, grp in enumerate(plan):
            wait(gi)
            old = nrows
            have |= set(grp)
            nrows = max([nrows] + [(k + 1) * 128 for c, k in grp if c == "x"])
            if nrows > old:
                xn_sc[old // 2:nrows // 2, :] = _bits(_layernorm(x_v[old:nrows, :]))
            for hi in (old, nrows):
                for p in range(npair):
                    if ("u", p) in have and done[p] < hi:
                        f0, f1 = p * 128, (p + 1) * 128
                        up(gate(done[p], hi, f0, f1), done[p], hi, f0, f1)
                        done[p] = hi
        assert nrows == T0
        for t in (1, 2, 0):
            _permute_cols(wqkv_v[:, t * D:(t + 1) * D].astype(F32).T, wqkv_p, t * D, tmp.at[t])
            if t > 0:
                proj(xn_rows(0, T0), t)
        wait(len(plan))
        proj(xn_rows(0, T0), 0, 0, 1)
        ffn_tail(xn_rows(0, T0))
        proj(xn_rows(0, T0), 0, 1, NT)
        _permute_rows(wo_v[...].astype(F32), wo_p, tmp.at[3])
        g = gate(0, T0, FC, F0)
        y = down(T0, 0, FC)
        up(g, 0, T0, FC, F0)
        attention(T0, T0, True)
        y = down(T0, FC, F) + y
        finish(0, T0, y)
        wait(len(plan) + 1)

        def body(i, carry):
            row0 = pl.multiple_of(T0 + i * TM, 128)
            nxt = pl.multiple_of(jnp.minimum(row0 + TM, S - TM), 128)
            xnp = gather(QR, TM // (2 * NCHAIN))
            proj(_bf16(xnp), 0)
            ffn_tail(_bf16(xnp))
            proj(_bf16(xnp), 1)
            proj(_bf16(xnp), 2)
            xn_sc[0:TM // 2, :] = xnp
            up(gate(0, TM, 0, F0), 0, TM, 0, F0)
            attention(TM, nxt, False)
            finish(row0, TM, down(TM, 0, F))
            return carry

        lax.fori_loop(0, (S - T0) // TM, body, 0)
        return carry_

    lax.fori_loop(0, z_sm[0] + 1, whole, 0)

    pltpu.make_async_copy(o_v, o_hbm, out_sem.at[0]).wait()


@jax.jit
def pallas_parallel_sum__sliding_local_dilated__geglu_ffn__prompt_kernel(
    A_x: jax.Array,
    A_wqkv: jax.Array,
    A_wo: jax.Array,
    B_x: jax.Array,
    B_w_gate: jax.Array,
    B_w_up: jax.Array,
    B_w_down: jax.Array,
):
    B, S, D = A_x.shape
    F = B_w_gate.shape[1]
    assert B == 1 and D == H * DH and (S - T0) % TM == 0 and S > T0 + TM
    NT = D // 128
    out = pl.pallas_call(
        _kernel,
        in_specs=[pl.BlockSpec(memory_space=pl.ANY)] * 6,
        out_specs=pl.BlockSpec(memory_space=pl.ANY),
        out_shape=jax.ShapeDtypeStruct((S, D), A_x.dtype),
        scratch_shapes=[
            pltpu.VMEM((S, D), BF16),
            pltpu.VMEM((S, D), BF16),
            pltpu.VMEM((D, 3 * D), BF16),
            pltpu.VMEM((D, D), BF16),
            pltpu.VMEM((F, D), BF16),
            pltpu.VMEM((F, D), BF16),
            pltpu.VMEM((F, D), BF16),
            pltpu.VMEM((D // 2, 3 * D), U32),
            pltpu.VMEM((D // 2, D), U32),
            pltpu.VMEM((TX // 2, D), U32),
            pltpu.VMEM((NT, TX + HALO, 128), F32),
            pltpu.VMEM((NT, TX + HALO, 128), F32),
            pltpu.VMEM((TX // 2, F), U32),
            pltpu.VMEM((4, NT, H * PITCH, 128), F32),
            pltpu.SMEM((1,), jnp.int32),
            pltpu.SemaphoreType.DMA((len(PLAN) + 2,)),
            pltpu.SemaphoreType.DMA((1,)),
        ] + [pltpu.VMEM((NT, SPARE + QPAD, 128), U32)
             for _ in range(NCHAIN)],
        compiler_params=pltpu.CompilerParams(
            vmem_limit_bytes=100 * 1024 * 1024,
            disable_bounds_checks=True,
            disable_semaphore_checks=True),
    )(A_x.reshape(S, D), A_wqkv, A_wo, B_w_gate.T, B_w_up.T, B_w_down)
    return out.reshape(B, S, D)
```

```python
import functools

import jax
import jax.numpy as jnp
from jax import lax
import jax.experimental.pallas as pl
import jax.experimental.pallas.tpu as pltpu

H = 32
DH = 16
W = 8
DIL = 2
HALO = 16
PITCH = 20
T0 = 768
TM = 640
TX = max(T0, TM)
RC = 8
LNR = 16
NCHAIN = 2
QR = TX // NCHAIN
SPARE = QR + TM // (2 * NCHAIN)
TRIG = 3
OR = 64
PIECE = {"x": 64, "g": 128, "u": 128}
PLAN = [["x0", "x1"], ["x2", "x3", "x4", "x5"], ["g0", "u0"], ["g1", "u1", "x6", "x7", "x8"],
        ["x9", "x10", "x11", "g2", "g3", "u2", "u3"], ["g4", "g5", "u4", "u5", "w0"]]
LOG2E = 1.4426950408889634
QSCALE = (DH ** -0.5) * LOG2E
GC1 = 0.7978845608028654
GC2 = GC1 * 0.044715
NT_DIMS = (((1,), (1,)), ((), ()))
F32 = jnp.float32
BF16 = jnp.bfloat16
U32 = jnp.uint32


def _bits(x):
    return pltpu.bitcast(x, U32)


def _bf16(x):
    return pltpu.bitcast(x, BF16)


def _f32(x):
    return pltpu.bitcast(x, F32)


def _geglu2(g, u):
    t = jnp.tanh(g * (GC1 + GC2 * (g * g)))
    gu = g * u
    return gu + gu * t


def _layernorm(x):
    x = x.astype(F32)
    m = jnp.mean(x, axis=-1, keepdims=True)
    xc = x - m
    var = jnp.mean(xc * xc, axis=-1, keepdims=True)
    return (xc * lax.rsqrt(var + 1e-5)).astype(BF16)


def _scatter_heads(src, tmp):
    for j in range(src.shape[1] // 128):
        for h in range(H):
            tmp[j, h * PITCH:h * PITCH + DH, :] = src[h * DH:(h + 1) * DH, j * 128:(j + 1) * 128]


def _permute_rows(src, dst_ref, tmp):
    _scatter_heads(src, tmp)
    for d in range(DH):
        for j in range(src.shape[1] // 128):
            dst_ref[d * H // 2:(d + 1) * H // 2, j * 128:(j + 1) * 128] = _bits(
                tmp[j, pl.ds(d, H, stride=PITCH), :].astype(BF16))


def _permute_cols(src_t, dst_ref, col0, tmp):
    _scatter_heads(src_t, tmp)
    dpt = 128 // H
    for c in range(DH // dpt):
        for j in range(src_t.shape[1] // 128):
            blk = jnp.concatenate(
                [tmp[j, pl.ds(c * dpt + d, H, stride=PITCH), :] for d in range(dpt)], axis=0)
            dst_ref[j * 64:(j + 1) * 64, col0 + c * 128:col0 + (c + 1) * 128] = _bits(
                blk.T.astype(BF16))


def _split(x, nrows):
    n = x.shape[0] // (NCHAIN * nrows)
    x = x.reshape(n, NCHAIN, nrows, 128)
    return [x[:, b].reshape(n * nrows, 128) for b in range(NCHAIN)]


def _merge(xs, nrows):
    n = xs[0].shape[0] // nrows
    x = jnp.concatenate([x.reshape(n, 1, nrows, 128) for x in xs], axis=1)
    return x.reshape(n * NCHAIN * nrows, 128)


def _attn_chunk(qa, k_sc, v_sc, z, g, b, masked):
    nt = k_sc.shape[0]
    r0 = (g * NCHAIN + b) * RC
    lr = g * RC
    buf = qa[b]
    qs = [_f32(buf[j, pl.ds(z + lr, RC), :]) for j in range(nt)]
    win = [pl.ds(r0 + (HALO - DIL * w), RC) for w in range(W)]
    ls = []
    for w in range(W):
        p = functools.reduce(jnp.add, [qs[j] * k_sc[j, win[w], :] for j in range(nt)])
        p = ((p + pltpu.roll(p, 32, 1)) + pltpu.roll(p, 64, 1)) + pltpu.roll(p, 96, 1)
        if masked and r0 < DIL * w:
            pos = r0 + lax.broadcasted_iota(jnp.int32, (RC, 128), 0)
            p = jnp.where(pos >= DIL * w, p, -1e9 * LOG2E)
        ls.append(p)
        if w == TRIG:
            qa[(b + 1) % NCHAIN][0, SPARE:SPARE + RC, :] = _bits(p)
    mx = functools.reduce(jnp.maximum, ls)
    es = [jnp.exp2(l - mx) for l in ls]
    den = functools.reduce(jnp.add, es)
    inv = pl.reciprocal(den, approx=True)
    inv = inv * (2.0 - den * inv)
    for j in range(nt):
        acc = functools.reduce(jnp.add, [es[w] * v_sc[j, win[w], :] for w in range(W)])
        buf[j, pl.ds(lr, RC), :] = _bits(acc * inv)


def _kernel(x_hbm, wqkv_hbm, wo_hbm, wg_hbm, wu_hbm, wd_hbm, o_hbm,
            x_v, o_v, wqkv_v, wo_v, wg_v, wu_v, wd_v, wqkv_p, wo_p,
            xn_sc, k_sc, v_sc, h_sc, tmp, z_sm, in_sem, out_sem, *qa):
    S, D = x_v.shape
    F = wg_v.shape[0]
    NT = D // 128
    F0 = F // 128 * 128
    FB = F - F0

    plan = [[(nm[0], int(nm[1:])) for nm in g] for g in PLAN]
    npair = max(k for g in plan for c, k in g if c == "u") + 1
    FC = npair * 128
    arrs = {"x": (x_hbm, x_v), "g": (wg_hbm, wg_v), "u": (wu_hbm, wu_v)}

    def rows(c, a, b):
        return (arrs[c][0].at[a:b], arrs[c][1].at[a:b])

    def merged(grp):
        runs = []
        for c, k in grp:
            if runs and runs[-1][0] == c and runs[-1][2] == k:
                runs[-1][2] = k + 1
            else:
                runs.append([c, k, k + 1])
        return [(wqkv_hbm, wqkv_v) if c == "w" else rows(c, a * PIECE[c], b * PIECE[c])
                for c, a, b in runs]

    groups = [merged(g) for g in plan]
    groups += [[rows("g", FC, F), rows("u", FC, F), rows("x", T0, T0 + TM),
                (wd_hbm, wd_v), (wo_hbm, wo_v)],
               [rows("x", T0 + TM, S)]]
    copies = [[pltpu.make_async_copy(src, dst, in_sem.at[gi]) for src, dst in grp]
              for gi, grp in enumerate(groups)]
    for grp in copies:
        for cp in grp:
            cp.start()
    z_sm[0] = 0

    def wait(gi):
        for cp in copies[gi]:
            cp.wait()

    def xn_rows(a, b):
        return _bf16(xn_sc[a // 2:b // 2, :])

    def gate(a, b, f0, f1):
        return lax.dot_general(xn_rows(a, b), wg_v[f0:f1, :], NT_DIMS, preferred_element_type=F32)

    def up(g, a, b, f0, f1):
        u = lax.dot_general(xn_rows(a, b), wu_v[f0:f1, :], NT_DIMS, preferred_element_type=F32)
        h_sc[a // 2:b // 2, f0:f1] = _bits(_geglu2(g, u).astype(BF16))

    def ffn_tail(xn):
        tm = xn.shape[0]
        w = jnp.concatenate([wg_v[F0:F, :], wu_v[F0:F, :]], axis=0)
        rt = lax.dot_general(w, xn, NT_DIMS, preferred_element_type=F32)
        ht = _geglu2(rt[0:FB], rt[FB:2 * FB])
        h = jnp.concatenate([ht, jnp.zeros((128 - FB, tm), F32)], axis=0).T
        h_sc[0:tm // 2, F0:F] = _bits(h.astype(BF16))[:, 0:FB]

    def down(tm, f0, f1):
        return jnp.dot(_bf16(h_sc[0:tm // 2, f0:f1]), wd_v[f0:f1, :], preferred_element_type=F32)

    def proj(xn, t, j0=0, j1=NT):
        tm = xn.shape[0]
        y = jnp.dot(xn, _bf16(wqkv_p[:, t * D + j0 * 128:t * D + j1 * 128]),
                    preferred_element_type=F32)
        for j in range(j0, j1):
            yj = y[:, (j - j0) * 128:(j - j0 + 1) * 128]
            if t == 0:
                for b, part in enumerate(_split(_bits(yj * QSCALE), RC)):
                    qa[b][j, 0:tm // NCHAIN, :] = part
            else:
                (k_sc if t == 1 else v_sc)[j, HALO:HALO + tm, :] = yj

    def gather(row0, n):
        return jnp.concatenate(
            [_merge([qa[b][j, row0:row0 + n, :] for b in range(NCHAIN)], RC) for j in range(NT)],
            axis=1)

    def attention(tm, next_row0, first):
        z = z_sm[0]

        def step(i, with_ln, masked=False):
            for lb in range(NCHAIN):
                g = i * NCHAIN + lb
                for b in range(NCHAIN):
                    _attn_chunk(qa, k_sc, v_sc, z, g, b, masked)
                if with_ln:
                    r = pl.multiple_of(next_row0 + g * LNR, LNR)
                    xn = _bits(_layernorm(x_v[pl.ds(r, LNR), :]))
                    for j in range(NT):
                        qa[lb][j, pl.ds(QR + i * (LNR // 2), LNR // 2), :] = (
                            xn[:, j * 128:(j + 1) * 128])

        def run(lo, hi, with_ln):
            def body(i, carry):
                step(i, with_ln)
                return carry
            if lo < hi:
                lax.fori_loop(lo, hi, body, 0, unroll=True)

        n_ln, n_all = TM // (LNR * NCHAIN), tm // (RC * NCHAIN * NCHAIN)
        if first:
            step(0, True, masked=True)
        run(1 if first else 0, n_ln, True)
        run(n_ln, n_all, False)
        k_sc[:, 0:HALO, :] = k_sc[:, tm:tm + HALO, :]
        v_sc[:, 0:HALO, :] = v_sc[:, tm:tm + HALO, :]

    def finish(row0, tm, y):
        a = _f32(gather(0, tm // NCHAIN)).astype(BF16)
        y = jnp.dot(a, _bf16(wo_p[...]), preferred_element_type=F32) + 0.5 * y

        def emit(a0, a1, c0, c1):
            idx = (pl.ds(row0 + a0, a1 - a0), pl.ds(c0, c1 - c0))
            o_v[idx] = (x_v[idx].astype(F32) + y[a0:a1, c0:c1]).astype(o_v.dtype)
            pltpu.make_async_copy(o_v.at[idx], o_hbm.at[idx], out_sem.at[0]).start()

        emit(0, tm, 0, D // 2)
        emit(0, tm, D // 2, D - 128)
        for a0 in range(0, tm, OR):
            emit(a0, a0 + OR, D - 128, D)

    def whole(i_, carry_):
        k_sc[:, 0:HALO, :] = jnp.zeros((NT, HALO, 128), F32)
        v_sc[:, 0:HALO, :] = jnp.zeros((NT, HALO, 128), F32)
        nrows = 0
        have = set()
        done = [0] * npair
        for gi, grp in enumerate(plan):
            wait(gi)
            old = nrows
            have |= set(grp)
            nrows = max([nrows] + [(k + 1) * PIECE[c] for c, k in grp if c == "x"])
            if nrows > old:
                xn_sc[old // 2:nrows // 2, :] = _bits(_layernorm(x_v[old:nrows, :]))
            for hi in (old, nrows):
                for p in range(npair):
                    if ("u", p) in have and done[p] < hi:
                        f0, f1 = p * 128, (p + 1) * 128
                        up(gate(done[p], hi, f0, f1), done[p], hi, f0, f1)
                        done[p] = hi
        assert nrows == T0
        for t in (1, 2, 0):
            _permute_cols(wqkv_v[:, t * D:(t + 1) * D].astype(F32).T, wqkv_p, t * D, tmp.at[t])
            if t > 0:
                proj(xn_rows(0, T0), t)
        wait(len(plan))
        proj(xn_rows(0, T0), 0, 0, 1)
        ffn_tail(xn_rows(0, T0))
        proj(xn_rows(0, T0), 0, 1, NT)
        _permute_rows(wo_v[...].astype(F32), wo_p, tmp.at[3])
        g = gate(0, T0, FC, F0)
        y = down(T0, 0, FC)
        up(g, 0, T0, FC, F0)
        attention(T0, T0, True)
        y = down(T0, FC, F) + y
        finish(0, T0, y)
        wait(len(plan) + 1)

        def body(i, carry):
            row0 = pl.multiple_of(T0 + i * TM, 128)
            nxt = pl.multiple_of(jnp.minimum(row0 + TM, S - TM), 128)
            xnp = gather(QR, TM // (2 * NCHAIN))
            proj(_bf16(xnp), 0)
            ffn_tail(_bf16(xnp))
            proj(_bf16(xnp), 1)
            proj(_bf16(xnp), 2)
            xn_sc[0:TM // 2, :] = xnp
            up(gate(0, TM, 0, F0), 0, TM, 0, F0)
            attention(TM, nxt, False)
            finish(row0, TM, down(TM, 0, F))
            return carry

        lax.fori_loop(0, (S - T0) // TM, body, 0)
        return carry_

    lax.fori_loop(0, z_sm[0] + 1, whole, 0)

    pltpu.make_async_copy(o_v, o_hbm, out_sem.at[0]).wait()


@jax.jit
def pallas_parallel_sum__sliding_local_dilated__geglu_ffn__prompt_kernel(
    A_x: jax.Array,
    A_wqkv: jax.Array,
    A_wo: jax.Array,
    B_x: jax.Array,
    B_w_gate: jax.Array,
    B_w_up: jax.Array,
    B_w_down: jax.Array,
):
    B, S, D = A_x.shape
    F = B_w_gate.shape[1]
    assert B == 1 and D == H * DH and (S - T0) % TM == 0 and S > T0 + TM
    NT = D // 128
    out = pl.pallas_call(
        _kernel,
        in_specs=[pl.BlockSpec(memory_space=pl.ANY)] * 6,
        out_specs=pl.BlockSpec(memory_space=pl.ANY),
        out_shape=jax.ShapeDtypeStruct((S, D), A_x.dtype),
        scratch_shapes=[
            pltpu.VMEM((S, D), BF16),
            pltpu.VMEM((S, D), BF16),
            pltpu.VMEM((D, 3 * D), BF16),
            pltpu.VMEM((D, D), BF16),
            pltpu.VMEM((F, D), BF16),
            pltpu.VMEM((F, D), BF16),
            pltpu.VMEM((F, D), BF16),
            pltpu.VMEM((D // 2, 3 * D), U32),
            pltpu.VMEM((D // 2, D), U32),
            pltpu.VMEM((TX // 2, D), U32),
            pltpu.VMEM((NT, TX + HALO, 128), F32),
            pltpu.VMEM((NT, TX + HALO, 128), F32),
            pltpu.VMEM((TX // 2, F), U32),
            pltpu.VMEM((4, NT, (H + 2) * PITCH, 128), F32),
            pltpu.SMEM((1,), jnp.int32),
            pltpu.SemaphoreType.DMA((len(PLAN) + 2,)),
            pltpu.SemaphoreType.DMA((1,)),
        ] + [pltpu.VMEM((NT, SPARE + RC, 128), U32)
             for _ in range(NCHAIN)],
        compiler_params=pltpu.CompilerParams(
            vmem_limit_bytes=100 * 1024 * 1024,
            disable_bounds_checks=True,
            disable_semaphore_checks=True),
    )(A_x.reshape(S, D), A_wqkv, A_wo, B_w_gate.T, B_w_up.T, B_w_down)
    return out.reshape(B, S, D)
```

```python
import functools

import jax
import jax.numpy as jnp
from jax import lax
import jax.experimental.pallas as pl
import jax.experimental.pallas.tpu as pltpu

H = 32
DH = 16
W = 8
DIL = 2
HALO = 16
PITCH = 36
TM = 1024
RC = 8
NCHAIN = 2
QR = TM // NCHAIN
QPAD = RC
TRIG = 3
COV = 256
RSTEP = 256
OR = 64
PIECE = {"x": 64, "g": 128, "u": 128}
PLAN = [[("x", 0, 2)], [("x", 2, 5)], [("g", 0, 1), ("u", 0, 1)],
        [("g", 1, 2), ("u", 1, 2), ("x", 5, 7)],
        [("g", 2, 3), ("u", 2, 3), ("x", 7, 12)],
        [("g", 3, 4), ("u", 3, 4), ("x", 12, 32)]]
LOG2E = 1.4426950408889634
QSCALE = (DH ** -0.5) * LOG2E
GC1 = 0.7978845608028654
GC2 = GC1 * 0.044715
NT_DIMS = (((1,), (1,)), ((), ()))
F32 = jnp.float32
BF16 = jnp.bfloat16
U32 = jnp.uint32


def _bits(x):
    return pltpu.bitcast(x, U32)


def _bf16(x):
    return pltpu.bitcast(x, BF16)


def _f32(x):
    return pltpu.bitcast(x, F32)


def _geglu2(g, u):
    t = jnp.tanh(g * (GC1 + GC2 * (g * g)))
    gu = g * u
    return gu + gu * t


def _layernorm(x):
    x = x.astype(F32)
    m = jnp.mean(x, axis=-1, keepdims=True)
    xc = x - m
    var = jnp.mean(xc * xc, axis=-1, keepdims=True)
    return (xc * lax.rsqrt(var + 1e-5)).astype(BF16)


def _scatter_heads(src, tmp):
    for j in range(src.shape[1] // 128):
        for h in range(H):
            tmp[j, pl.ds(h, DH, stride=PITCH), :] = src[h * DH:(h + 1) * DH, j * 128:(j + 1) * 128]


def _permute_rows(src, dst_ref, tmps, z):
    for j in range(src.shape[1] // 128):
        _scatter_heads(src[:, j * 128:(j + 1) * 128], tmps[j])
        blk = jnp.concatenate([tmps[j][0, pl.ds(z + d * PITCH, H), :] for d in range(DH)], axis=0)
        dst_ref[:, j * 128:(j + 1) * 128] = _bits(blk.astype(BF16))


def _permute_cols(src_t, dst_ref, col0, tmp, z):
    _scatter_heads(src_t, tmp)
    dpt = 128 // H
    for c in range(DH // dpt):
        for j in range(src_t.shape[1] // 128):
            blk = jnp.concatenate(
                [tmp[j, pl.ds(z + (c * dpt + d) * PITCH, H), :] for d in range(dpt)], axis=0)
            dst_ref[j * 64:(j + 1) * 64, col0 + c * 128:col0 + (c + 1) * 128] = _bits(
                blk.T.astype(BF16))


def _split(x, nrows):
    n = x.shape[0] // (NCHAIN * nrows)
    x = x.reshape(n, NCHAIN, nrows, 128)
    return [x[:, b].reshape(n * nrows, 128) for b in range(NCHAIN)]


def _merge(xs, nrows):
    n = xs[0].shape[0] // nrows
    x = jnp.concatenate([x.reshape(n, 1, nrows, 128) for x in xs], axis=1)
    return x.reshape(n * NCHAIN * nrows, 128)


def _attn_chunk(qa, k_sc, v_sc, z, g, b, row0):
    nt = k_sc.shape[0]
    r0 = (g * NCHAIN + b) * RC
    lr = g * RC
    buf = qa[b]
    qs = [_f32(buf[j, pl.ds(z + lr, RC), :]) for j in range(nt)]
    win = [pl.ds(r0 + (HALO - DIL * w), RC) for w in range(W)]
    ls = []
    for w in range(W):
        p = functools.reduce(jnp.add, [qs[j] * k_sc[j, win[w], :] for j in range(nt)])
        p = ((p + pltpu.roll(p, 32, 1)) + pltpu.roll(p, 64, 1)) + pltpu.roll(p, 96, 1)
        if row0 is not None and r0 < DIL * w:
            pos = row0 + r0 + lax.broadcasted_iota(jnp.int32, (RC, 128), 0)
            p = jnp.where(pos >= DIL * w, p, -1e9 * LOG2E)
        ls.append(p)
        if w == TRIG:
            qa[(b + 1) % NCHAIN][0, QR:QR + RC, :] = _bits(p)
    mx = functools.reduce(jnp.maximum, ls)
    es = [jnp.exp2(l - mx) for l in ls]
    den = functools.reduce(jnp.add, es)
    inv = pl.reciprocal(den, approx=True)
    inv = inv * (2.0 - den * inv)
    for j in range(nt):
        acc = functools.reduce(jnp.add, [es[w] * v_sc[j, win[w], :] for w in range(W)])
        buf[j, pl.ds(lr, RC), :] = _bits(acc * inv)


def _kernel(x_hbm, wqkv_hbm, wo_hbm, wg_hbm, wu_hbm, wd_hbm, o_hbm,
            x_v, o_v, wqkv_v, wo_v, wg_v, wu_v, wd_v, wqkv_p, wo_p,
            xn_sc, k_sc, v_sc, h_sc, z_sm, in_sem, out_sem, *bufs):
    S, D = x_v.shape
    F = wg_v.shape[0]
    NT = D // 128
    F0 = F // 128 * 128
    FB = F - F0
    qa, tmp_qkv, tmp_o = bufs[:NCHAIN], bufs[NCHAIN:NCHAIN + 3], bufs[NCHAIN + 3:]

    npair = max(b for grp in PLAN for c, a, b in grp if c == "u")
    FC = npair * 128
    arrs = {"x": (x_hbm, x_v), "g": (wg_hbm, wg_v), "u": (wu_hbm, wu_v)}

    def rows(c, a, b):
        return (arrs[c][0].at[a:b], arrs[c][1].at[a:b])

    groups = [[rows(c, a * PIECE[c], b * PIECE[c]) for c, a, b in grp] for grp in PLAN]
    groups.append([rows("g", FC, F), rows("u", FC, F), (wqkv_hbm, wqkv_v),
                   (wd_hbm, wd_v), (wo_hbm, wo_v)])
    copies = [[pltpu.make_async_copy(src, dst, in_sem.at[gi]) for src, dst in grp]
              for gi, grp in enumerate(groups)]
    for grp in copies:
        for cp in grp:
            cp.start()
    z_sm[0] = 0

    def wait(gi):
        for cp in copies[gi]:
            cp.wait()

    def xn_rows(r, n):
        return _bf16(xn_sc[pl.ds(r, n // 2), :])

    def gate(r, n, f0, f1):
        return lax.dot_general(xn_rows(r, n), wg_v[f0:f1, :], NT_DIMS, preferred_element_type=F32)

    def up(g, r, n, f0, f1):
        u = lax.dot_general(xn_rows(r, n), wu_v[f0:f1, :], NT_DIMS, preferred_element_type=F32)
        h_sc[pl.ds(r, n // 2), f0:f1] = _bits(_geglu2(g, u).astype(BF16))

    def ffn_tail(r):
        w = jnp.concatenate([wg_v[F0:F, :], wu_v[F0:F, :]], axis=0)
        rt = lax.dot_general(w, xn_rows(r, TM), NT_DIMS, preferred_element_type=F32)
        ht = _geglu2(rt[0:FB], rt[FB:2 * FB])
        h = jnp.concatenate([ht, jnp.zeros((128 - FB, TM), F32)], axis=0).T
        h_sc[pl.ds(r, TM // 2), F0:F] = _bits(h.astype(BF16))[:, 0:FB]

    def down(r, f0, f1):
        return jnp.dot(_bf16(h_sc[pl.ds(r, TM // 2), f0:f1]), wd_v[f0:f1, :],
                       preferred_element_type=F32)

    def proj(r, t):
        y = jnp.dot(xn_rows(r, TM), _bf16(wqkv_p[:, t * D:(t + 1) * D]),
                    preferred_element_type=F32)
        for j in range(NT):
            yj = y[:, j * 128:(j + 1) * 128]
            if t == 0:
                for b, part in enumerate(_split(_bits(yj * QSCALE), RC)):
                    qa[b][j, 0:QR, :] = part
            else:
                (k_sc if t == 1 else v_sc)[j, HALO:HALO + TM, :] = yj

    def attention(row0):
        z = z_sm[0]

        def step(g, mask_row0):
            for b in range(NCHAIN):
                _attn_chunk(qa, k_sc, v_sc, z, g, b, mask_row0)

        def body(g, carry):
            step(g, None)
            return carry

        step(0, row0)
        lax.fori_loop(1, TM // (RC * NCHAIN), body, 0, unroll=True)
        k_sc[:, 0:HALO, :] = k_sc[:, TM:TM + HALO, :]
        v_sc[:, 0:HALO, :] = v_sc[:, TM:TM + HALO, :]

    def finish(row0, y):
        a = jnp.concatenate(
            [_merge([qa[b][j, 0:QR, :] for b in range(NCHAIN)], RC) for j in range(NT)], axis=1)
        y = jnp.dot(_f32(a).astype(BF16), _bf16(wo_p[...]), preferred_element_type=F32) + 0.5 * y

        def emit(a0, a1, c0, c1):
            idx = (pl.ds(row0 + a0, a1 - a0), pl.ds(c0, c1 - c0))
            o_v[idx] = (x_v[idx].astype(F32) + y[a0:a1, c0:c1]).astype(o_v.dtype)
            pltpu.make_async_copy(o_v.at[idx], o_hbm.at[idx], out_sem.at[0]).start()

        emit(0, TM, 0, D // 2)
        emit(0, TM, D // 2, D - 128)
        for a0 in range(0, TM, OR):
            emit(a0, a0 + OR, D - 128, D)

    def whole(i_, carry_):
        k_sc[:, 0:HALO, :] = jnp.zeros((NT, HALO, 128), F32)
        v_sc[:, 0:HALO, :] = jnp.zeros((NT, HALO, 128), F32)
        nrows = npairs = 0
        done = [0] * npair
        for gi, grp in enumerate(PLAN):
            wait(gi)
            old = nrows
            nrows = max([nrows] + [b * PIECE[c] for c, a, b in grp if c == "x"])
            npairs = max([npairs] + [b for c, a, b in grp if c == "u"])
            if nrows > old:
                xn_sc[old // 2:nrows // 2, :] = _bits(_layernorm(x_v[old:nrows, :]))
            for hi in [old] + list(range(old + RSTEP, nrows, RSTEP)) + [nrows]:
                for p in range(npairs):
                    if done[p] < hi:
                        f0, f1 = p * 128, (p + 1) * 128
                        r, n = done[p] // 2, hi - done[p]
                        up(gate(r, n, f0, f1), r, n, f0, f1)
                        done[p] = hi
        assert nrows == S
        wait(len(PLAN))

        def body(i, carry):
            row0 = pl.multiple_of(i * TM, TM)
            r = pl.multiple_of(i * (TM // 2), TM // 2)
            y = down(r, 0, COV)
            for t in (1, 2, 0):
                _permute_cols(wqkv_v[:, t * D:(t + 1) * D].astype(F32).T, wqkv_p, t * D,
                              tmp_qkv[t], z_sm[0])
                proj(r, t)
                if t == 1:
                    ffn_tail(r)
            _permute_rows(wo_v[...].astype(F32), wo_p, tmp_o, z_sm[0])
            g = gate(r, TM, FC, F0)
            y = down(r, COV, FC) + y
            up(g, r, TM, FC, F0)
            attention(row0)
            y = down(r, FC, F) + y
            finish(row0, y)
            return carry

        lax.fori_loop(0, S // TM, body, 0)
        return carry_

    lax.fori_loop(0, z_sm[0] + 1, whole, 0)

    pltpu.make_async_copy(o_v, o_hbm, out_sem.at[0]).wait()


@jax.jit
def pallas_parallel_sum__sliding_local_dilated__geglu_ffn__prompt_kernel(
    A_x: jax.Array,
    A_wqkv: jax.Array,
    A_wo: jax.Array,
    B_x: jax.Array,
    B_w_gate: jax.Array,
    B_w_up: jax.Array,
    B_w_down: jax.Array,
):
    B, S, D = A_x.shape
    F = B_w_gate.shape[1]
    assert B == 1 and D == H * DH and S % TM == 0
    NT = D // 128
    stage_rows = (DH + 1) * PITCH + 4
    out = pl.pallas_call(
        _kernel,
        in_specs=[pl.BlockSpec(memory_space=pl.ANY)] * 6,
        out_specs=pl.BlockSpec(memory_space=pl.ANY),
        out_shape=jax.ShapeDtypeStruct((S, D), A_x.dtype),
        scratch_shapes=[
            pltpu.VMEM((S, D), BF16),
            pltpu.VMEM((S, D), BF16),
            pltpu.VMEM((D, 3 * D), BF16),
            pltpu.VMEM((D, D), BF16),
            pltpu.VMEM((F, D), BF16),
            pltpu.VMEM((F, D), BF16),
            pltpu.VMEM((F, D), BF16),
            pltpu.VMEM((D // 2, 3 * D), U32),
            pltpu.VMEM((D // 2, D), U32),
            pltpu.VMEM((S // 2, D), U32),
            pltpu.VMEM((NT, TM + HALO, 128), F32),
            pltpu.VMEM((NT, TM + HALO, 128), F32),
            pltpu.VMEM((S // 2, F), U32),
            pltpu.SMEM((1,), jnp.int32),
            pltpu.SemaphoreType.DMA((len(PLAN) + 1,)),
            pltpu.SemaphoreType.DMA((1,)),
        ]
        + [pltpu.VMEM((NT, QR + QPAD, 128), U32) for _ in range(NCHAIN)]
        + [pltpu.VMEM((NT, stage_rows, 128), F32) for _ in range(3)]
        + [pltpu.VMEM((1, stage_rows, 128), F32) for _ in range(NT)],
        compiler_params=pltpu.CompilerParams(
            vmem_limit_bytes=100 * 1024 * 1024,
            disable_bounds_checks=True,
            disable_semaphore_checks=True),
    )(A_x.reshape(S, D), A_wqkv, A_wo, B_w_gate.T, B_w_up.T, B_w_down)
    return out.reshape(B, S, D)
```
